```python
import os as _os
_os.environ.setdefault("JAX_PLATFORMS", "cpu")
import jax
import jax.numpy as jnp

def _softmax(x, axis=-1):
    return jax.nn.softmax(x, axis=axis)
def _gelu(x):
    return jax.nn.gelu(x, approximate=True)
def _silu(x):
    return jax.nn.silu(x)
def _sigmoid(x):
    return jax.nn.sigmoid(x)
def _layernorm(x, axis=-1, eps=1e-5):
    m = jnp.mean(x, axis=axis, keepdims=True)
    v = jnp.var(x, axis=axis, keepdims=True)
    return (x - m) / jnp.sqrt(v + eps)
def _scatter_add(tgt, idx, src, axis=0):
    return tgt.at[idx].add(src)
def _segment_sum(src, seg, n):
    return jax.ops.segment_sum(src, seg, n)
class _Rng:
    def __init__(self, key):
        self._k = key
    def _next(self):
        self._k, sub = jax.random.split(self._k)
        return sub
    def normal(self, shape):
        return jax.random.normal(self._next(), shape, dtype=jnp.bfloat16)
    def randint(self, lo, hi, shape):
        return jax.random.randint(self._next(), shape, lo, hi, dtype=jnp.int32)
    def uniform(self, shape, lo=0.0, hi=1.0):
        return jax.random.uniform(self._next(), shape, jnp.bfloat16, lo, hi)
    def permutation(self, n):
        return jax.random.permutation(self._next(), n)


kernel_name = 'interleave_layers__gqa_block_cached__dense_activation_silu__decode'

def setup_inputs():
    _rng = _Rng(jax.random.key(int.from_bytes(__import__("os").urandom(4), "little")))
    _w = (lambda a: (lambda t: t.astype(jnp.bfloat16) if jnp.issubdtype(t.dtype, jnp.floating) else t)(jnp.asarray(a)))
    def _A_setup():
        B, Sq, D = 2, 1, 512
        Hq, Hkv, Sk, Dh = 32, 8, 8192, 128
        assert Hq % Hkv == 0, (Hq, Hkv)
        return {
            "x": _w((lambda *s: _rng.normal(s) * 0.1)(B, Sq, D)),
            "k_cache": _w((lambda *s: _rng.normal(s) * 0.8)(B, Hkv, Sk, Dh)),
            "v_cache": _w((lambda *s: _rng.normal(s) * 1.6)(B, Hkv, Sk, Dh)),
            "wq": _w((lambda *s: _rng.normal(s) * 0.8)(D, Hq * Dh) * (D ** -0.5)),
            "wo": _w((lambda *s: _rng.normal(s) * 1.6)(Hq * Dh, D) * ((Hq * Dh) ** -0.5)),
        }
    _A_in = _A_setup()

    def _B_setup():
        B, S, D, F = 2, 1, 512, 1792
        return {
            "x": _w((lambda *s: _rng.normal(s) * 0.1)(B, S, D)),
            "w1": _w((lambda *s: _rng.normal(s) * 0.4)(D, F) * (D ** -0.5)),
            "w2": _w((lambda *s: _rng.normal(s) * 0.4)(F, D) * (F ** -0.5)),
        }
    _B_in = _B_setup()

    return {
        "A_x": _A_in["x"],
        "A_k_cache": _A_in["k_cache"],
        "A_v_cache": _A_in["v_cache"],
        "A_wq": _A_in["wq"],
        "A_wo": _A_in["wo"],
        "B_x": _B_in["x"],
        "B_w1": _B_in["w1"],
        "B_w2": _B_in["w2"],
    }

def reference(A_x, A_k_cache, A_v_cache, A_wq, A_wo, B_x, B_w1, B_w2):
    def _A_ref(x, k_cache, v_cache, wq, wo):
        B, Sq, D = x.shape
        Hq, Dh = 32, 128
        Hkv = k_cache.shape[1]
        rep = Hq // Hkv
        q = (lambda x, *d: x.transpose(*d))((x @ wq).reshape(B, Sq, Hq, Dh), 0, 2, 1, 3)
        k = jnp.repeat(k_cache, rep, axis=1)
        v = jnp.repeat(v_cache, rep, axis=1)
        scores = jnp.einsum("bhqd,bhkd->bhqk", q, k) * (Dh ** -0.5)
        p = _softmax(scores, axis=-1)
        o = jnp.einsum("bhqk,bhkd->bhqd", p, v)
        return (lambda x, *d: x.transpose(*d))(o, 0, 2, 1, 3).reshape(B, Sq, Hq * Dh) @ wo

    def _B_ref(x, w1, w2):
        h = jnp.einsum("bsd,df->bsf", x, w1)
        h = _silu(h)
        out = jnp.einsum("bsf,fd->bsd", h, w2)
        return out

    x = A_x
    x = x + _A_ref(_layernorm(x, axis=-1), A_k_cache, A_v_cache, A_wq, A_wo)
    x = x + _B_ref(_layernorm(x, axis=-1), B_w1, B_w2)
    x = x + _A_ref(_layernorm(x, axis=-1), A_k_cache, A_v_cache, A_wq, A_wo)
    x = x + _B_ref(_layernorm(x, axis=-1), B_w1, B_w2)
    return x
```

```python
import functools
import jax
import jax.numpy as jnp
from jax import lax
import jax.experimental.pallas as pl
import jax.experimental.pallas.tpu as pltpu

B, D = 2, 512
HQ, HKV, SK, DH = 32, 8, 8192, 128
REP = HQ // HKV
F = 1792
EPS = 1e-5
SCALE = DH ** -0.5
f32, bf16, u32 = jnp.float32, jnp.bfloat16, jnp.uint32
L = 128
TK = 2048
NVL = 4
VL = SK // NVL
NSEM_B = HKV + (HKV - 1) + NVL
NQM = 2
NOM = 2
PIN = 3
NFV = 6
NFM = F // L - NFV
SPLIT = 4096
HW = REP * DH


def _center(x):
    m = jnp.mean(x, axis=-1, keepdims=True)
    xc = x - m
    v = jnp.mean(xc * xc, axis=-1, keepdims=True)
    return xc, m, lax.rsqrt(v + EPS)


def _silu(h):
    hh = 0.5 * h
    return hh + hh * jnp.tanh(hh)


def _dot(a, b32):
    return jnp.dot(a, pltpu.bitcast(b32, bf16), preferred_element_type=f32)


def _dot_nt(a, b):
    return lax.dot_general(a, b, (((1,), (1,)), ((), ())), preferred_element_type=f32)


def _sublane_allsum(x):
    x = x + pltpu.roll(x, 4, 0)
    x = x + pltpu.roll(x, 2, 0)
    return x + pltpu.roll(x, 1, 0)


def _kernel(x_hbm, k_hbm, v_hbm, wq_hbm, wo_hbm, w1_hbm, w2_hbm, o_ref,
            k_scr, v_scr, kt_scr, wq_s, wo_s, w1_s, w2_s, wq_r, wo_r, w1_r, w2_r, wq32, wot32, w1t32, w2f32,
            q_scr, s_scr, p_scr, l_scr, cs1_scr, csq_scr, x_ref, sem):
    def kcopy(b, h):
        return pltpu.make_async_copy(k_hbm.at[b * HKV + h], k_scr.at[h], sem.at[4 + b * NSEM_B + h])

    def vcopy(b, h):
        return pltpu.make_async_copy(v_hbm.at[b * HKV + h], v_scr.at[b * HKV + h], sem.at[4 + b * NSEM_B + HKV + h])

    def vlast(b, c):
        i = b * HKV + HKV - 1
        return pltpu.make_async_copy(v_hbm.at[i, pl.ds(c * VL, VL)], v_scr.at[i, pl.ds(c * VL, VL)],
                                     sem.at[4 + b * NSEM_B + 2 * HKV - 1 + c])

    def start_kv(b):
        for h in range(HKV):
            kcopy(b, h).start()
        for h in range(HKV - 1):
            vcopy(b, h).start()
        for c in range(NVL):
            vlast(b, c).start()

    wcopies = [pltpu.make_async_copy(a, b, sem.at[i]) for i, (a, b) in enumerate(
        [(wq_hbm, wq_s), (wo_hbm, wo_s), (w1_hbm, w1_s), (w2_hbm, w2_s)])]
    xcopy = pltpu.make_async_copy(x_hbm, x_ref, sem.at[4 + B * NSEM_B])

    xcopy.start()
    for c in wcopies:
        c.start()
    start_kv(0)

    v32 = v_scr.bitcast(u32)
    row = lax.broadcasted_iota(jnp.int32, (8, DH), 0)
    rowr = row % REP
    eye = (lax.broadcasted_iota(jnp.int32, (DH, DH), 0)
           == lax.broadcasted_iota(jnp.int32, (DH, DH), 1)).astype(bf16)

    def retile(ws, wr, r_lo, r_hi, cols):
        rb = 256
        for jj, j in enumerate(cols):
            def rbody(i, _, jj=jj, j=j):
                r0 = pl.multiple_of(r_lo + i * rb, rb)
                wr[jj, pl.ds(pl.multiple_of(i * (rb // 2), rb // 2), rb // 2), :] = pltpu.bitcast(
                    ws[pl.ds(r0, rb), j * L:(j + 1) * L], u32)
                return 0
            lax.fori_loop(0, (r_hi - r_lo) // rb, rbody, 0)

    wcopies[0].wait()
    retile(wq_s, wq_r, 0, D, range(NQM * REP))
    ones8 = jnp.ones((8, D), bf16)
    csq_scr[...] = jnp.dot(ones8, wq_s[:, :NQM * HW], preferred_element_type=f32)
    for j in range(NQM * REP, HQ):
        wq32[j - NQM * REP] = _dot_nt(eye, wq_s[:, j * L:(j + 1) * L])
    wcopies[1].wait()
    retile(wo_s, wo_r, (HKV - NOM) * HW, HKV * HW, range(D // L))

    def tbody(i, _):
        r0 = pl.multiple_of(i * L, L)
        wot32[pl.ds(r0, L), :] = wo_s[pl.ds(r0, L), :].astype(f32)
        return 0
    lax.fori_loop(0, (HKV - NOM) * REP, tbody, 0)
    wcopies[2].wait()
    retile(w1_s, w1_r, 0, D, range(NFM))
    cs1_scr[...] = jnp.dot(ones8, w1_s[:, :NFM * L], preferred_element_type=f32)
    for j in range(NFV):
        t = _dot_nt(eye, w1_s[:, (NFM + j) * L:(NFM + j + 1) * L])
        w1t32[j] = t - jnp.mean(t, axis=1, keepdims=True)
    wcopies[3].wait()

    def w2body(i, _):
        w2_r[i] = pltpu.bitcast(w2_s[pl.ds(pl.multiple_of(i * L, L), L), :], u32)
        return 0
    lax.fori_loop(0, NFM, w2body, 0)
    for j in range(NFV):
        w2f32[j] = w2_s[(NFM + j) * L:(NFM + j + 1) * L, :].astype(f32)

    def qselect(c):
        return jnp.where(rowr == 0, c[0], jnp.where(rowr == 1, c[1], jnp.where(rowr == 2, c[2], c[3])))

    def expand(o):
        return jnp.concatenate([jnp.where(row == r, o, 0.0) for r in range(REP)], axis=1).astype(bf16)

    def oproj_mxu(o, h):
        oh = expand(o)
        hh = (h - (HKV - NOM)) * HW // 2
        return jnp.concatenate([_dot(oh, wo_r[j, hh:hh + HW // 2, :]) for j in range(D // L)], axis=1)

    def dep(x, t):
        return jnp.where(t != t, t, x)

    def qhead_vpu(xc, h):
        cs = []
        for r in range(REP):
            w = wq32[(h - NQM) * REP + r]
            prod = w.reshape(L // 8, 8, D) * xc[None]
            part = prod[:, :, 0:L]
            for cb in range(1, D // L):
                part = part + prod[:, :, cb * L:(cb + 1) * L]
            t = part.reshape(L, L).T
            cs.append(_sublane_allsum(jnp.sum(t.reshape(L // 8, 8, L), axis=0)))
        return qselect(cs)

    def oproj_vpu(o, h, acc):
        for r in range(REP):
            ob = jnp.broadcast_to(o[r:r + 1, :], (L, L)).T
            w = wot32[(h * REP + r) * L:(h * REP + r + 1) * L, :]
            prod = jnp.concatenate([ob] * (D // L), axis=1) * w
            t = jnp.sum(prod.reshape(L // 8, 8, D), axis=0)
            acc = t if acc is None else acc + t
        return acc

    def ln_stats(x8, c):
        xb = x8.astype(bf16)
        xs = xb.astype(f32) - c
        ms = jnp.mean(xs, axis=-1, keepdims=True)
        v = jnp.maximum(jnp.mean(xs * xs, axis=-1, keepdims=True) - ms * ms, 0.0)
        return xb, xs - ms, ms + c, lax.rsqrt(v + EPS)

    def ffn(x8, c):
        xb, _, m, rs = ln_stats(x8, c)
        hs = []
        for j in range(NFM):
            hdn = (_dot(xb, w1_r[j]) - m * cs1_scr[:, j * L:(j + 1) * L]) * rs
            hs.append(_silu(hdn).astype(bf16))
        y = _dot(hs[0], w2_r[0])
        for j in range(1, NFM):
            y = y + _dot(hs[j], w2_r[j])
        xr = xb.astype(f32)
        yv = None
        for j in range(NFV):
            prod = w1t32[j].reshape(L // 8, 8, D) * xr[None]
            part = prod[:, :, 0:L]
            for cb in range(1, D // L):
                part = part + prod[:, :, cb * L:(cb + 1) * L]
            hdn = jnp.sum(part, axis=-1, keepdims=True) * rs[None]
            hdn = _silu(hdn)
            t = jnp.sum(w2f32[j].reshape(L // 8, 8, D) * hdn, axis=0)
            yv = t if yv is None else yv + t
        return y + _sublane_allsum(yv), m

    lo = row < REP

    def softmax(s):
        sp = jnp.concatenate(
            [jnp.where(lo, s[:, 2 * j * L:(2 * j + 1) * L], s[:, (2 * j + 1) * L:(2 * j + 2) * L])
             for j in range(SK // (2 * L))], axis=1)
        m = jnp.broadcast_to(jnp.max(sp, axis=1, keepdims=True), (8, L))
        m = jnp.maximum(m, pltpu.roll(m, REP, 0))
        p = jnp.exp(sp - jnp.concatenate([m] * (SK // (2 * L)), axis=1))
        l = jnp.broadcast_to(jnp.sum(p, axis=1, keepdims=True), (8, L))
        l = l + pltpu.roll(l, REP, 0)
        tiles = []
        for j in range(SK // (2 * L)):
            pj = p[:, j * L:(j + 1) * L]
            tiles += [jnp.where(lo, pj, 0.0), jnp.where(lo, 0.0, pj)]
        return jnp.concatenate(tiles, axis=1).astype(bf16), l

    def fold(o8, l):
        return (o8 + pltpu.roll(o8, REP, 0)) / l

    def batch(b, carry):
        xf = x_ref[...].astype(f32)
        x8 = jnp.where(b == 0, jnp.broadcast_to(xf[0:1], (8, D)), jnp.broadcast_to(xf[1:2], (8, D)))
        xc, m, rs = _center(x8)
        q8 = jnp.dot(xc.astype(bf16), wq_s[...], preferred_element_type=f32) * (rs * SCALE)
        for h in range(HKV):
            q_scr[h] = qselect([q8[:, (REP * h + r) * DH:(REP * h + r + 1) * DH] for r in range(REP)])

        def kbody(h, _):
            kcopy(b, h).wait()
            qh = q_scr[h]
            lhs = jnp.concatenate([jnp.concatenate([qh, qh], axis=0).astype(bf16), eye], axis=0)

            def chunk(c, _):
                off = pl.multiple_of(c * TK, TK)
                r = _dot_nt(lhs, k_scr[h, pl.ds(off, TK), :])
                s_scr[:, pl.ds(off, TK)] = r[:8]
                kt_scr[h, :, pl.ds(off, TK)] = pltpu.bitcast(r[16:].astype(bf16), u32)
                return 0
            lax.fori_loop(0, SK // TK, chunk, 0)
            p, l = softmax(s_scr[...])
            l_scr[h] = l
            p_scr[h] = p
            return 0
        lax.fori_loop(0, HKV, kbody, 0)

        @pl.when(b + 1 < B)
        def _():
            start_kv(b + 1)

        def vbody(h, acc):
            vcopy(b, h).wait()
            o = fold(_dot(p_scr[h], v32[b * HKV + h]), l_scr[h])
            wo_h = wo_s[pl.ds(pl.multiple_of(h * HW, HW), HW), :]
            return acc + jnp.dot(expand(o), wo_h, preferred_element_type=f32)
        acc = lax.fori_loop(0, HKV - 1, vbody, jnp.zeros((8, D), f32))
        h = HKV - 1
        o = jnp.zeros((8, DH), f32)
        for c in range(NVL):
            vlast(b, c).wait()
            o = o + _dot(p_scr[h, :, c * VL:(c + 1) * VL], v32[b * HKV + h, c * VL // 2:(c + 1) * VL // 2, :])
        acc = acc + oproj_mxu(fold(o, l_scr[h]), h)
        x8 = x8 + _sublane_allsum(acc)
        y, m = ffn(x8, m)
        x8 = x8 + y

        xb, xc, m, rs = ln_stats(x8, m)
        rq = rs * SCALE
        qs = {}
        for h in range(NQM):
            qraw = qselect([_dot(xb, wq_r[REP * h + r]) for r in range(REP)])
            qcs = qselect([csq_scr[:, (REP * h + r) * L:(REP * h + r + 1) * L] for r in range(REP)])
            qs[h] = (qraw - m * qcs) * rq
        ss, os_, accs = {}, {}, {}

        def qk(h):
            pin = accs.get(h - PIN)
            if pin is None:
                return _dot(qs[h].astype(bf16), kt_scr[h])
            q2 = qs[h]
            for j in range(D // L):
                q2 = dep(q2, pin[:, j * L:(j + 1) * L])
            return jnp.concatenate([_dot(qs[h].astype(bf16), kt_scr[h, :, :SPLIT]),
                                    _dot(q2.astype(bf16), kt_scr[h, :, SPLIT:])], axis=1)

        ss[0] = qk(0)
        acc = None
        for h in range(HKV):
            if h + 1 < HKV:
                if h + 1 not in qs:
                    qs[h + 1] = qhead_vpu(xc, h + 1) * rq
                ss[h + 1] = qk(h + 1)
            p, l = softmax(ss[h])
            os_[h] = fold(_dot(p, v32[b * HKV + h]), l)
            if h < HKV - NOM:
                acc = oproj_vpu(os_[h], h, acc)
                accs[h] = acc
        for h in range(HKV - NOM, HKV):
            acc = acc + oproj_mxu(os_[h], h)
        x8 = x8 + _sublane_allsum(acc)
        x8 = x8 + ffn(x8, m)[0]
        return jnp.where(lax.broadcasted_iota(jnp.int32, (8, D), 0) == b, x8, carry)

    xcopy.wait()
    res = lax.fori_loop(0, B, batch, jnp.zeros((8, D), f32))
    o_ref[...] = res[:B].astype(o_ref.dtype)


@jax.jit
def pallas_interleave_layers__gqa_block_cached__dense_activation_silu__decode_kernel(A_x, A_k_cache, A_v_cache, A_wq, A_wo, B_x, B_w1, B_w2):
    k = A_k_cache.reshape(B * HKV, SK, DH)
    v = A_v_cache.reshape(B * HKV, SK, DH)
    any_spec = pl.BlockSpec(memory_space=pl.ANY)
    return pl.pallas_call(
        _kernel,
        out_shape=jax.ShapeDtypeStruct((B, D), A_x.dtype),
        in_specs=[any_spec] * 7,
        out_specs=pl.BlockSpec(memory_space=pltpu.VMEM),
        scratch_shapes=[
            pltpu.VMEM((HKV, SK, DH), bf16),
            pltpu.VMEM((B * HKV, SK, DH), bf16),
            pltpu.VMEM((HKV, DH // 2, SK), u32),
            pltpu.VMEM((D, HQ * DH), bf16),
            pltpu.VMEM((HQ * DH, D), bf16),
            pltpu.VMEM((D, F), bf16),
            pltpu.VMEM((F, D), bf16),
            pltpu.VMEM((NQM * REP, D // 2, L), u32),
            pltpu.VMEM((D // L, NOM * HW // 2, L), u32),
            pltpu.VMEM((NFM, D // 2, L), u32),
            pltpu.VMEM((NFM, L // 2, D), u32),
            pltpu.VMEM(((HKV - NQM) * REP, L, D), f32),
            pltpu.VMEM(((HKV - NOM) * HW, D), f32),
            pltpu.VMEM((NFV, L, D), f32),
            pltpu.VMEM((NFV, L, D), f32),
            pltpu.VMEM((HKV, 8, DH), f32),
            pltpu.VMEM((8, SK), f32),
            pltpu.VMEM((HKV, 8, SK), bf16),
            pltpu.VMEM((HKV, 8, DH), f32),
            pltpu.VMEM((8, NFM * L), f32),
            pltpu.VMEM((8, NQM * HW), f32),
            pltpu.VMEM((B, D), bf16),
            pltpu.SemaphoreType.DMA((5 + B * NSEM_B,)),
        ],
        compiler_params=pltpu.CompilerParams(vmem_limit_bytes=120 * 1024 * 1024, disable_semaphore_checks=True),
    )(A_x.reshape(B, D), k, v, A_wq, A_wo, B_w1, B_w2).reshape(B, 1, D)
```

```python
import jax
import jax.numpy as jnp
from jax import lax
import jax.experimental.pallas as pl
import jax.experimental.pallas.tpu as pltpu

B, D = 2, 512
HQ, HKV, SK, DH = 32, 8, 8192, 128
REP = HQ // HKV
F = 1792
EPS = 1e-5
SCALE = DH ** -0.5
f32, bf16, u32 = jnp.float32, jnp.bfloat16, jnp.uint32
L = 128
HW = REP * DH
TK = 2048
VCH = (4096, 2048, 1024, 1024)
VOFF = tuple(sum(VCH[:i]) for i in range(len(VCH)))
NSEM_B = HKV + (HKV - 1) + len(VCH)
NQM = 2
NOM = 2
PIN = 3
SPLIT = 4096
NFV = 6
NFM = F // L - NFV
SB, SH = B - 1, HKV - 2
SROWS = 1024
NSC = SK // SROWS


def _silu(h):
    hh = 0.5 * h
    return hh + hh * jnp.tanh(hh)


def _dot(a, b32):
    return jnp.dot(a, pltpu.bitcast(b32, bf16), preferred_element_type=f32)


def _dot_nt(a, b):
    return lax.dot_general(a, b, (((1,), (1,)), ((), ())), preferred_element_type=f32)


def _sublane_allsum(x):
    x = x + pltpu.roll(x, 4, 0)
    x = x + pltpu.roll(x, 2, 0)
    return x + pltpu.roll(x, 1, 0)


def _kernel(x_hbm, k_hbm, v_hbm, wq_hbm, wo_hbm, w1_hbm, w2_hbm, o_ref,
            k_scr, v_scr, kt_scr, v32, wq_s, wo_s, w1_s, w2_s, wq_r, wo_r, w1_r, w2_r,
            wqt32, wo32, w1t32, w2f32,
            q_scr, s_scr, p_scr, l_scr, cs1_scr, csq_scr, x_ref, sm, sem, ssem):
    def kcopy(b, h):
        return pltpu.make_async_copy(k_hbm.at[b * HKV + h], k_scr.at[h], sem.at[4 + b * NSEM_B + h])

    def vcopy(b, h):
        return pltpu.make_async_copy(v_hbm.at[b * HKV + h], v_scr.at[h], sem.at[4 + b * NSEM_B + HKV + h])

    def vlast(b, c):
        h = HKV - 1
        return pltpu.make_async_copy(v_hbm.at[b * HKV + h, pl.ds(VOFF[c], VCH[c])],
                                     v_scr.at[h, pl.ds(VOFF[c], VCH[c])],
                                     sem.at[4 + b * NSEM_B + 2 * HKV - 1 + c])

    def start_k(b):
        for h in range(HKV):
            kcopy(b, h).start()

    def start_v(b, skip=None):
        for h in range(HKV - 1):
            if h != skip:
                vcopy(b, h).start()
        for c in range(len(VCH)):
            vlast(b, c).start()

    def side_in(c, buf):
        return pltpu.make_async_copy(v_hbm.at[SB * HKV + SH, pl.ds(c * SROWS, SROWS)], sm.at[buf], ssem.at[buf])

    def side_out(c, buf):
        return pltpu.make_async_copy(sm.at[buf], v_scr.at[HKV, pl.ds(c * SROWS, SROWS)], ssem.at[buf])

    def pump(k):
        j = k - 1
        buf = j % 2
        c = 2 * (j // 4) + buf

        @pl.when(jnp.logical_and(j < 2 * NSC, (j // 2) % 2 == 0))
        def _():
            side_in(c, buf).wait()
            side_out(c, buf).start()

        @pl.when(jnp.logical_and(j < 2 * NSC, (j // 2) % 2 == 1))
        def _():
            side_out(c, buf).wait()

            @pl.when(c + 2 < NSC)
            def _():
                side_in(c + 2, buf).start()

    wcopies = [pltpu.make_async_copy(a, b, sem.at[i]) for i, (a, b) in enumerate(
        [(wq_hbm, wq_s), (wo_hbm, wo_s), (w1_hbm, w1_s), (w2_hbm, w2_s)])]
    xcopy = pltpu.make_async_copy(x_hbm, x_ref, sem.at[4 + B * NSEM_B])

    xcopy.start()
    side_in(0, 0).start()
    side_in(1, 1).start()
    for c in wcopies:
        c.start()
    start_k(0)
    start_v(0)

    row = lax.broadcasted_iota(jnp.int32, (8, DH), 0)
    rowr = row % REP
    lo = row < REP
    eye = (lax.broadcasted_iota(jnp.int32, (DH, DH), 0)
           == lax.broadcasted_iota(jnp.int32, (DH, DH), 1)).astype(bf16)
    ones8 = jnp.ones((8, D), bf16)

    def retile(ws, wr, r_lo, r_hi, cols):
        rb = 256
        for j in cols:
            def rbody(i, _, j=j):
                r0 = pl.multiple_of(r_lo + i * rb, rb)
                wr[j, pl.ds(pl.multiple_of(i * (rb // 2), rb // 2), rb // 2), :] = pltpu.bitcast(
                    ws[pl.ds(r0, rb), j * L:(j + 1) * L], u32)
                return 0
            lax.fori_loop(0, (r_hi - r_lo) // rb, rbody, 0)

    wcopies[0].wait()
    retile(wq_s, wq_r, 0, D, range(NQM * REP))
    csq_scr[...] = jnp.dot(ones8, wq_s[:, :NQM * HW], preferred_element_type=f32)
    for j in range(NQM * REP, HQ):
        wqt32[j - NQM * REP] = _dot_nt(eye, wq_s[:, j * L:(j + 1) * L])
    pump(jnp.int32(1))
    wcopies[1].wait()
    retile(wo_s, wo_r, (HKV - NOM) * HW, HKV * HW, range(D // L))

    def obody(i, _):
        r0 = pl.multiple_of(i * L, L)
        wo32[pl.ds(r0, L), :] = wo_s[pl.ds(r0, L), :].astype(f32)
        return 0
    lax.fori_loop(0, (HKV - NOM) * REP, obody, 0)
    wcopies[2].wait()
    retile(w1_s, w1_r, 0, D, range(NFM))
    cs1_scr[...] = jnp.dot(ones8, w1_s[:, :NFM * L], preferred_element_type=f32)
    for j in range(NFV):
        t = _dot_nt(eye, w1_s[:, (NFM + j) * L:(NFM + j + 1) * L])
        w1t32[j] = t - jnp.mean(t, axis=1, keepdims=True)
    pump(jnp.int32(2))
    wcopies[3].wait()

    def w2body(i, _):
        w2_r[i] = pltpu.bitcast(w2_s[pl.ds(pl.multiple_of(i * L, L), L), :], u32)
        return 0
    lax.fori_loop(0, NFM, w2body, 0)
    for j in range(NFV):
        w2f32[j] = w2_s[(NFM + j) * L:(NFM + j + 1) * L, :].astype(f32)

    def qselect(c):
        return jnp.where(rowr == 0, c[0], jnp.where(rowr == 1, c[1], jnp.where(rowr == 2, c[2], c[3])))

    def expand(o):
        return jnp.concatenate([jnp.where(row == r, o, 0.0) for r in range(REP)], axis=1).astype(bf16)

    def oproj_mxu(o, h):
        oh = expand(o)
        hh = (h - (HKV - NOM)) * HW // 2
        return jnp.concatenate([_dot(oh, wo_r[j, hh:hh + HW // 2, :]) for j in range(D // L)], axis=1)

    def dep(x, t):
        return jnp.where(t != t, t, x)

    def lane_fold(w, x):
        prod = w.reshape(L // 8, 8, D) * x[None]
        part = prod[:, :, 0:L]
        for cb in range(1, D // L):
            part = part + prod[:, :, cb * L:(cb + 1) * L]
        return part

    def qhead_vpu(xc, h):
        cs = []
        for r in range(REP):
            t = lane_fold(wqt32[(h - NQM) * REP + r], xc).reshape(L, L).T
            cs.append(_sublane_allsum(jnp.sum(t.reshape(L // 8, 8, L), axis=0)))
        return qselect(cs)

    def oproj_vpu(o, h, acc):
        for r in range(REP):
            ob = jnp.broadcast_to(o[r:r + 1, :], (L, L)).T
            w = wo32[(h * REP + r) * L:(h * REP + r + 1) * L, :]
            prod = jnp.concatenate([ob] * (D // L), axis=1) * w
            t = jnp.sum(prod.reshape(L // 8, 8, D), axis=0)
            acc = t if acc is None else acc + t
        return acc

    def ln_stats(x8, c):
        xb = x8.astype(bf16)
        xs = xb.astype(f32) - c
        ms = jnp.mean(xs, axis=-1, keepdims=True)
        v = jnp.maximum(jnp.mean(xs * xs, axis=-1, keepdims=True) - ms * ms, 0.0)
        return xb, xs - ms, ms + c, lax.rsqrt(v + EPS)

    def ffn(x8, c):
        xb, _, m, rs = ln_stats(x8, c)
        hs = []
        for j in range(NFM):
            hdn = (_dot(xb, w1_r[j]) - m * cs1_scr[:, j * L:(j + 1) * L]) * rs
            hs.append(_silu(hdn).astype(bf16))
        y = _dot(hs[0], w2_r[0])
        for j in range(1, NFM):
            y = y + _dot(hs[j], w2_r[j])
        xr = xb.astype(f32)
        yv = None
        for j in range(NFV):
            hdn = jnp.sum(lane_fold(w1t32[j], xr), axis=-1, keepdims=True) * rs[None]
            t = jnp.sum(w2f32[j].reshape(L // 8, 8, D) * _silu(hdn), axis=0)
            yv = t if yv is None else yv + t
        return y + _sublane_allsum(yv), m

    def softmax(s):
        sp = jnp.concatenate(
            [jnp.where(lo, s[:, 2 * j * L:(2 * j + 1) * L], s[:, (2 * j + 1) * L:(2 * j + 2) * L])
             for j in range(SK // (2 * L))], axis=1)
        m = jnp.broadcast_to(jnp.max(sp, axis=1, keepdims=True), (8, L))
        m = jnp.maximum(m, pltpu.roll(m, REP, 0))
        p = jnp.exp(sp - jnp.concatenate([m] * (SK // (2 * L)), axis=1))
        l = jnp.broadcast_to(jnp.sum(p, axis=1, keepdims=True), (8, L))
        l = l + pltpu.roll(l, REP, 0)
        tiles = []
        for j in range(SK // (2 * L)):
            pj = p[:, j * L:(j + 1) * L]
            tiles += [jnp.where(lo, pj, 0.0), jnp.where(lo, 0.0, pj)]
        return jnp.concatenate(tiles, axis=1).astype(bf16), l

    def fold(o8, l):
        return (o8 + pltpu.roll(o8, REP, 0)) / l

    def batch(b, carry):
        @pl.when(b > 0)
        def _():
            start_v(b, SH)
            pump(2 + 9 * b)

        xf = x_ref[...].astype(f32)
        x8 = jnp.where(b == 0, jnp.broadcast_to(xf[0:1], (8, D)), jnp.broadcast_to(xf[1:2], (8, D)))
        m = jnp.mean(x8, axis=-1, keepdims=True)
        xc = x8 - m
        rs = lax.rsqrt(jnp.mean(xc * xc, axis=-1, keepdims=True) + EPS)
        q8 = jnp.dot(xc.astype(bf16), wq_s[...], preferred_element_type=f32) * (rs * SCALE)
        for h in range(HKV):
            q_scr[h] = qselect([q8[:, (REP * h + r) * DH:(REP * h + r + 1) * DH] for r in range(REP)])

        def kbody(h, _):
            kcopy(b, h).wait()

            @pl.when(h % 2 == 1)
            def _():
                pump(3 + 9 * b + h // 2)
            qh = q_scr[h]
            lhs = jnp.concatenate([jnp.concatenate([qh, qh], axis=0).astype(bf16), eye], axis=0)

            def chunk(c, _):
                off = pl.multiple_of(c * TK, TK)
                r = _dot_nt(lhs, k_scr[h, pl.ds(off, TK), :])
                s_scr[:, pl.ds(off, TK)] = r[:8]
                kt_scr[h, :, pl.ds(off, TK)] = pltpu.bitcast(r[16:].astype(bf16), u32)
                return 0
            lax.fori_loop(0, SK // TK, chunk, 0)
            p, l = softmax(s_scr[...])
            l_scr[h] = l
            p_scr[h] = p
            return 0
        lax.fori_loop(0, HKV, kbody, 0)

        @pl.when(b + 1 < B)
        def _():
            start_k(b + 1)

        def vbody(h, acc):
            side = jnp.logical_and(b == SB, h == SH)

            @pl.when(jnp.logical_not(side))
            def _():
                vcopy(b, h).wait()

            @pl.when(h % 2 == 1)
            def _():
                pump(7 + 9 * b + h // 2)
            vv = pltpu.bitcast(v_scr[jnp.where(side, HKV, h)], u32)
            v32[h] = vv
            o = fold(_dot(p_scr[h], vv), l_scr[h])
            wo_h = wo_s[pl.ds(pl.multiple_of(h * HW, HW), HW), :]
            return acc + jnp.dot(expand(o), wo_h, preferred_element_type=f32)
        acc = lax.fori_loop(0, HKV - 1, vbody, jnp.zeros((8, D), f32))
        pump(10 + 9 * b)
        h = HKV - 1
        o = jnp.zeros((8, DH), f32)
        for c in range(len(VCH)):
            vlast(b, c).wait()
            vv = pltpu.bitcast(v_scr[h, VOFF[c]:VOFF[c] + VCH[c], :], u32)
            v32[h, VOFF[c] // 2:(VOFF[c] + VCH[c]) // 2, :] = vv
            o = o + _dot(p_scr[h, :, VOFF[c]:VOFF[c] + VCH[c]], vv)
        acc = acc + oproj_mxu(fold(o, l_scr[h]), h)
        x8 = x8 + _sublane_allsum(acc)
        y, m = ffn(x8, m)
        x8 = x8 + y

        xb, xc, m, rs = ln_stats(x8, m)
        rq = rs * SCALE
        qs, ss, os_, accs = {}, {}, {}, {}
        for h in range(NQM):
            qraw = qselect([_dot(xb, wq_r[REP * h + r]) for r in range(REP)])
            qcs = qselect([csq_scr[:, (REP * h + r) * L:(REP * h + r + 1) * L] for r in range(REP)])
            qs[h] = (qraw - m * qcs) * rq

        def qk(h):
            pin = accs.get(h - PIN)
            if pin is None:
                return _dot(qs[h].astype(bf16), kt_scr[h])
            q2 = qs[h]
            for j in range(D // L):
                q2 = dep(q2, pin[:, j * L:(j + 1) * L])
            return jnp.concatenate([_dot(qs[h].astype(bf16), kt_scr[h, :, :SPLIT]),
                                    _dot(q2.astype(bf16), kt_scr[h, :, SPLIT:])], axis=1)

        ss[0] = qk(0)
        acc = None
        for h in range(HKV):
            if h + 1 < HKV:
                if h + 1 not in qs:
                    qs[h + 1] = qhead_vpu(xc, h + 1) * rq
                ss[h + 1] = qk(h + 1)
            p, l = softmax(ss[h])
            os_[h] = fold(_dot(p, v32[h]), l)
            if h < HKV - NOM:
                acc = oproj_vpu(os_[h], h, acc)
                accs[h] = acc
        for h in range(HKV - NOM, HKV):
            acc = acc + oproj_mxu(os_[h], h)
        x8 = x8 + _sublane_allsum(acc)
        x8 = x8 + ffn(x8, m)[0]
        return jnp.where(lax.broadcasted_iota(jnp.int32, (8, D), 0) == b, x8, carry)

    xcopy.wait()
    res = lax.fori_loop(0, B, batch, jnp.zeros((8, D), f32))
    o_ref[...] = res[:B].astype(o_ref.dtype)


@jax.jit
def pallas_interleave_layers__gqa_block_cached__dense_activation_silu__decode_kernel(A_x, A_k_cache, A_v_cache, A_wq, A_wo, B_x, B_w1, B_w2):
    k = A_k_cache.reshape(B * HKV, SK, DH)
    v = A_v_cache.reshape(B * HKV, SK, DH)
    any_spec = pl.BlockSpec(memory_space=pl.ANY)
    return pl.pallas_call(
        _kernel,
        out_shape=jax.ShapeDtypeStruct((B, D), A_x.dtype),
        in_specs=[any_spec] * 7,
        out_specs=pl.BlockSpec(memory_space=pltpu.VMEM),
        scratch_shapes=[
            pltpu.VMEM((HKV, SK, DH), bf16),
            pltpu.VMEM((HKV + 1, SK, DH), bf16),
            pltpu.VMEM((HKV, DH // 2, SK), u32),
            pltpu.VMEM((HKV, SK // 2, DH), u32),
            pltpu.VMEM((D, HQ * DH), bf16),
            pltpu.VMEM((HQ * DH, D), bf16),
            pltpu.VMEM((D, F), bf16),
            pltpu.VMEM((F, D), bf16),
            pltpu.VMEM((NQM * REP, D // 2, L), u32),
            pltpu.VMEM((D // L, NOM * HW // 2, L), u32),
            pltpu.VMEM((NFM, D // 2, L), u32),
            pltpu.VMEM((NFM, L // 2, D), u32),
            pltpu.VMEM(((HKV - NQM) * REP, L, D), f32),
            pltpu.VMEM(((HKV - NOM) * HW, D), f32),
            pltpu.VMEM((NFV, L, D), f32),
            pltpu.VMEM((NFV, L, D), f32),
            pltpu.VMEM((HKV, 8, DH), f32),
            pltpu.VMEM((8, SK), f32),
            pltpu.VMEM((HKV, 8, SK), bf16),
            pltpu.VMEM((HKV, 8, DH), f32),
            pltpu.VMEM((8, NFM * L), f32),
            pltpu.VMEM((8, NQM * HW), f32),
            pltpu.VMEM((B, D), bf16),
            pltpu.SMEM((2, SROWS, DH), bf16),
            pltpu.SemaphoreType.DMA((5 + B * NSEM_B,)),
            pltpu.SemaphoreType.DMA((2,)),
        ],
        compiler_params=pltpu.CompilerParams(vmem_limit_bytes=120 * 1024 * 1024, disable_semaphore_checks=True),
    )(A_x.reshape(B, D), k, v, A_wq, A_wo, B_w1, B_w2).reshape(B, 1, D)
```

```python
import jax
import jax.numpy as jnp
from jax import lax
import jax.experimental.pallas as pl
import jax.experimental.pallas.tpu as pltpu

B, D = 2, 512
HQ, HKV, SK, DH = 32, 8, 8192, 128
REP = HQ // HKV
F = 1792
EPS = 1e-5
SCALE = DH ** -0.5
f32, bf16, u32 = jnp.float32, jnp.bfloat16, jnp.uint32
L = 128
HW = REP * DH
TK = 2048
XR = 768
VCH = (XR, 4096 - XR, 2048, 1024, 1024)
VORD = (1, 2, 3, 0, 4)
XH = 3
VOFF = tuple(sum(VCH[:i]) for i in range(len(VCH)))
NSEM_B = HKV + (HKV - 1) + len(VCH)
NQM = 1
NOM = 2
PIN = 3
SPLIT = 3072
NFV = 6
NFM = F // L - NFV
SB, SH = B - 1, HKV - 2
SROWS = 1024
NSC = SK // SROWS


def _silu(h):
    hh = 0.5 * h
    return hh + hh * jnp.tanh(hh)


def _dot(a, b32):
    return jnp.dot(a, pltpu.bitcast(b32, bf16), preferred_element_type=f32)


def _dot_nt(a, b):
    return lax.dot_general(a, b, (((1,), (1,)), ((), ())), preferred_element_type=f32)


def _sublane_allsum(x):
    x = x + pltpu.roll(x, 4, 0)
    x = x + pltpu.roll(x, 2, 0)
    return x + pltpu.roll(x, 1, 0)


def _kernel(x_hbm, k_hbm, v_hbm, wq_hbm, wo_hbm, w1_hbm, w2_hbm, o_ref,
            k_scr, v_scr, kt_scr, v32, wq_s, wo_s, w1_s, w2_s, wq_r, wo_r, w1_r, w2_r,
            wqt32, wo32, w1t32, w2f32,
            q_scr, s_scr, p_scr, l_scr, cs1_scr, csq_scr, x_ref, sm, sem, ssem):
    def kcopy(b, h):
        return pltpu.make_async_copy(k_hbm.at[b * HKV + h], k_scr.at[h], sem.at[4 + b * NSEM_B + h])

    def vcopy(b, h):
        return pltpu.make_async_copy(v_hbm.at[b * HKV + h], v_scr.at[h], sem.at[4 + b * NSEM_B + HKV + h])

    def vlast(b, c):
        h = HKV - 1
        return pltpu.make_async_copy(v_hbm.at[b * HKV + h, pl.ds(VOFF[c], VCH[c])],
                                     v_scr.at[h, pl.ds(VOFF[c], VCH[c])],
                                     sem.at[4 + b * NSEM_B + 2 * HKV - 1 + c])

    def start_k(b):
        for h in range(HKV):
            kcopy(b, h).start()

    def start_v(b, skip=None):
        for h in range(HKV - 1):
            if h != skip:
                vcopy(b, h).start()
        for c in VORD:
            if not (skip is not None and c == 0):
                vlast(b, c).start()

    def side_in(c, buf):
        return pltpu.make_async_copy(v_hbm.at[SB * HKV + SH, pl.ds(c * SROWS, SROWS)], sm.at[buf], ssem.at[buf])

    def side_out(c, buf):
        return pltpu.make_async_copy(sm.at[buf], v_scr.at[HKV, pl.ds(c * SROWS, SROWS)], ssem.at[buf])

    xtra_in = pltpu.make_async_copy(v_hbm.at[SB * HKV + HKV - 1, pl.ds(0, XR)], sm.at[0, pl.ds(0, XR)], ssem.at[0])
    xtra_out = pltpu.make_async_copy(sm.at[0, pl.ds(0, XR)], v_scr.at[HKV - 1, pl.ds(0, XR)], ssem.at[0])

    def pump(k):
        j = k - 1
        buf = j % 2
        c = 2 * (j // 4) + buf

        @pl.when(jnp.logical_and(j < 2 * NSC, (j // 2) % 2 == 0))
        def _():
            side_in(c, buf).wait()
            side_out(c, buf).start()

        @pl.when(jnp.logical_and(j < 2 * NSC, (j // 2) % 2 == 1))
        def _():
            side_out(c, buf).wait()

            @pl.when(c + 2 < NSC)
            def _():
                side_in(c + 2, buf).start()

            @pl.when(c + 2 == NSC)
            def _():
                xtra_in.start()

    wcopies = [pltpu.make_async_copy(a, b, sem.at[i]) for i, (a, b) in enumerate(
        [(wq_hbm, wq_s), (wo_hbm, wo_s), (w1_hbm, w1_s), (w2_hbm, w2_s)])]
    xcopy = pltpu.make_async_copy(x_hbm, x_ref, sem.at[4 + B * NSEM_B])

    xcopy.start()
    side_in(0, 0).start()
    side_in(1, 1).start()
    for c in wcopies:
        c.start()
    start_k(0)
    start_v(0)

    row = lax.broadcasted_iota(jnp.int32, (8, DH), 0)
    rowr = row % REP
    lo = row < REP
    eye = (lax.broadcasted_iota(jnp.int32, (DH, DH), 0)
           == lax.broadcasted_iota(jnp.int32, (DH, DH), 1)).astype(bf16)
    ones8 = jnp.ones((8, D), bf16)

    def retile(ws, wr, r_lo, r_hi, cols):
        rb = 256
        for j in cols:
            def rbody(i, _, j=j):
                r0 = pl.multiple_of(r_lo + i * rb, rb)
                wr[j, pl.ds(pl.multiple_of(i * (rb // 2), rb // 2), rb // 2), :] = pltpu.bitcast(
                    ws[pl.ds(r0, rb), j * L:(j + 1) * L], u32)
                return 0
            lax.fori_loop(0, (r_hi - r_lo) // rb, rbody, 0)

    wcopies[0].wait()
    retile(wq_s, wq_r, 0, D, range(NQM * REP))
    csq_scr[...] = jnp.dot(ones8, wq_s[:, :NQM * HW], preferred_element_type=f32)
    for j in range(NQM * REP, HQ):
        wqt32[j - NQM * REP] = _dot_nt(eye, wq_s[:, j * L:(j + 1) * L])
    pump(jnp.int32(1))
    wcopies[1].wait()
    retile(wo_s, wo_r, (HKV - NOM) * HW, HKV * HW, range(D // L))

    def obody(i, _):
        r0 = pl.multiple_of(i * L, L)
        wo32[pl.ds(r0, L), :] = wo_s[pl.ds(r0, L), :].astype(f32)
        return 0
    lax.fori_loop(0, (HKV - NOM) * REP, obody, 0)
    wcopies[2].wait()
    retile(w1_s, w1_r, 0, D, range(NFM))
    cs1_scr[...] = jnp.dot(ones8, w1_s[:, :NFM * L], preferred_element_type=f32)
    for j in range(NFV):
        t = _dot_nt(eye, w1_s[:, (NFM + j) * L:(NFM + j + 1) * L])
        w1t32[j] = t - jnp.mean(t, axis=1, keepdims=True)
    pump(jnp.int32(2))
    wcopies[3].wait()

    def w2body(i, _):
        w2_r[i] = pltpu.bitcast(w2_s[pl.ds(pl.multiple_of(i * L, L), L), :], u32)
        return 0
    lax.fori_loop(0, NFM, w2body, 0)
    for j in range(NFV):
        w2f32[j] = w2_s[(NFM + j) * L:(NFM + j + 1) * L, :].astype(f32)

    def qselect(c):
        return jnp.where(rowr == 0, c[0], jnp.where(rowr == 1, c[1], jnp.where(rowr == 2, c[2], c[3])))

    def expand(o):
        return jnp.concatenate([jnp.where(row == r, o, 0.0) for r in range(REP)], axis=1).astype(bf16)

    def oproj_mxu(o, h):
        oh = expand(o)
        hh = (h - (HKV - NOM)) * HW // 2
        return jnp.concatenate([_dot(oh, wo_r[j, hh:hh + HW // 2, :]) for j in range(D // L)], axis=1)

    def dep(x, t):
        return jnp.where(t != t, t, x)

    def lane_fold(w, x):
        prod = w.reshape(L // 8, 8, D) * x[None]
        part = prod[:, :, 0:L]
        for cb in range(1, D // L):
            part = part + prod[:, :, cb * L:(cb + 1) * L]
        return part

    def qhead_vpu(xc, h):
        cs = []
        for r in range(REP):
            t = lane_fold(wqt32[(h - NQM) * REP + r], xc).reshape(L, L).T
            cs.append(_sublane_allsum(jnp.sum(t.reshape(L // 8, 8, L), axis=0)))
        return qselect(cs)

    def oproj_vpu(o, h, acc):
        for r in range(REP):
            ob = jnp.broadcast_to(o[r:r + 1, :], (L, L)).T
            w = wo32[(h * REP + r) * L:(h * REP + r + 1) * L, :]
            prod = jnp.concatenate([ob] * (D // L), axis=1) * w
            t = jnp.sum(prod.reshape(L // 8, 8, D), axis=0)
            acc = t if acc is None else acc + t
        return acc

    def ln_stats(x8, c):
        xb = x8.astype(bf16)
        xs = xb.astype(f32) - c
        ms = jnp.mean(xs, axis=-1, keepdims=True)
        v = jnp.maximum(jnp.mean(xs * xs, axis=-1, keepdims=True) - ms * ms, 0.0)
        return xb, xs - ms, ms + c, lax.rsqrt(v + EPS)

    def ffn(x8, c):
        xb, _, m, rs = ln_stats(x8, c)
        hs = []
        for j in range(NFM):
            hdn = (_dot(xb, w1_r[j]) - m * cs1_scr[:, j * L:(j + 1) * L]) * rs
            hs.append(_silu(hdn).astype(bf16))
        y = _dot(hs[0], w2_r[0])
        for j in range(1, NFM):
            y = y + _dot(hs[j], w2_r[j])
        xr = xb.astype(f32)
        yv = None
        for j in range(NFV):
            hdn = jnp.sum(lane_fold(w1t32[j], xr), axis=-1, keepdims=True) * rs[None]
            t = jnp.sum(w2f32[j].reshape(L // 8, 8, D) * _silu(hdn), axis=0)
            yv = t if yv is None else yv + t
        return y + _sublane_allsum(yv), m

    def softmax(s):
        sp = jnp.concatenate(
            [jnp.where(lo, s[:, 2 * j * L:(2 * j + 1) * L], s[:, (2 * j + 1) * L:(2 * j + 2) * L])
             for j in range(SK // (2 * L))], axis=1)
        m = jnp.broadcast_to(jnp.max(sp, axis=1, keepdims=True), (8, L))
        m = jnp.maximum(m, pltpu.roll(m, REP, 0))
        p = jnp.exp(sp - jnp.concatenate([m] * (SK // (2 * L)), axis=1))
        l = jnp.broadcast_to(jnp.sum(p, axis=1, keepdims=True), (8, L))
        l = l + pltpu.roll(l, REP, 0)
        tiles = []
        for j in range(SK // (2 * L)):
            pj = p[:, j * L:(j + 1) * L]
            tiles += [jnp.where(lo, pj, 0.0), jnp.where(lo, 0.0, pj)]
        return jnp.concatenate(tiles, axis=1).astype(bf16), l

    def fold(o8, l):
        return (o8 + pltpu.roll(o8, REP, 0)) / l

    def batch(b, carry):
        @pl.when(b > 0)
        def _():
            start_v(b, SH)
            pump(2 + 9 * b)

        xf = x_ref[...].astype(f32)
        x8 = jnp.where(b == 0, jnp.broadcast_to(xf[0:1], (8, D)), jnp.broadcast_to(xf[1:2], (8, D)))
        m = jnp.mean(x8, axis=-1, keepdims=True)
        xc = x8 - m
        rs = lax.rsqrt(jnp.mean(xc * xc, axis=-1, keepdims=True) + EPS)
        q8 = jnp.dot(xc.astype(bf16), wq_s[...], preferred_element_type=f32) * (rs * SCALE)
        for h in range(HKV):
            q_scr[h] = qselect([q8[:, (REP * h + r) * DH:(REP * h + r + 1) * DH] for r in range(REP)])

        def kbody(h, _):
            kcopy(b, h).wait()

            @pl.when(h % 2 == 1)
            def _():
                pump(3 + 9 * b + h // 2)
            qh = q_scr[h]
            lhs = jnp.concatenate([jnp.concatenate([qh, qh], axis=0).astype(bf16), eye], axis=0)

            def chunk(c, _):
                off = pl.multiple_of(c * TK, TK)
                r = _dot_nt(lhs, k_scr[h, pl.ds(off, TK), :])
                s_scr[:, pl.ds(off, TK)] = r[:8]
                kt_scr[h, :, pl.ds(off, TK)] = pltpu.bitcast(r[16:].astype(bf16), u32)
                return 0
            lax.fori_loop(0, SK // TK, chunk, 0)
            p, l = softmax(s_scr[...])
            l_scr[h] = l
            p_scr[h] = p
            return 0
        lax.fori_loop(0, HKV, kbody, 0)

        @pl.when(b + 1 < B)
        def _():
            start_k(b + 1)

        def vbody(h, acc):
            side = jnp.logical_and(b == SB, h == SH)

            @pl.when(jnp.logical_not(side))
            def _():
                vcopy(b, h).wait()

            @pl.when(h % 2 == 1)
            def _():
                pump(7 + 9 * b + h // 2)

            @pl.when(jnp.logical_and(b == SB, h == XH))
            def _():
                xtra_in.wait()
                xtra_out.start()
            vv = pltpu.bitcast(v_scr[jnp.where(side, HKV, h)], u32)
            v32[h] = vv
            o = fold(_dot(p_scr[h], vv), l_scr[h])
            wo_h = wo_s[pl.ds(pl.multiple_of(h * HW, HW), HW), :]
            return acc + jnp.dot(expand(o), wo_h, preferred_element_type=f32)
        acc = lax.fori_loop(0, HKV - 1, vbody, jnp.zeros((8, D), f32))
        pump(10 + 9 * b)
        h = HKV - 1
        o = jnp.zeros((8, DH), f32)
        for c in VORD:
            if c == 0:
                @pl.when(b == SB)
                def _():
                    xtra_out.wait()

                @pl.when(b != SB)
                def _():
                    vlast(b, 0).wait()
            else:
                vlast(b, c).wait()
            vv = pltpu.bitcast(v_scr[h, VOFF[c]:VOFF[c] + VCH[c], :], u32)
            v32[h, VOFF[c] // 2:(VOFF[c] + VCH[c]) // 2, :] = vv
            o = o + _dot(p_scr[h, :, VOFF[c]:VOFF[c] + VCH[c]], vv)
        acc = acc + oproj_mxu(fold(o, l_scr[h]), h)
        x8 = x8 + _sublane_allsum(acc)
        y, m = ffn(x8, m)
        x8 = x8 + y

        xb, xc, m, rs = ln_stats(x8, m)
        rq = rs * SCALE
        qs, ss, os_, accs = {}, {}, {}, {}
        for h in range(NQM):
            qraw = qselect([_dot(xb, wq_r[REP * h + r]) for r in range(REP)])
            qcs = qselect([csq_scr[:, (REP * h + r) * L:(REP * h + r + 1) * L] for r in range(REP)])
            qs[h] = (qraw - m * qcs) * rq

        def qk(h):
            pin = accs.get(h - PIN)
            if pin is None:
                return _dot(qs[h].astype(bf16), kt_scr[h])
            q2 = qs[h]
            for j in range(D // L):
                q2 = dep(q2, pin[:, j * L:(j + 1) * L])
            return jnp.concatenate([_dot(qs[h].astype(bf16), kt_scr[h, :, :SPLIT]),
                                    _dot(q2.astype(bf16), kt_scr[h, :, SPLIT:])], axis=1)

        ss[0] = qk(0)
        acc = None
        for h in range(HKV):
            if h + 1 < HKV:
                if h + 1 not in qs:
                    qs[h + 1] = qhead_vpu(xc, h + 1) * rq
                ss[h + 1] = qk(h + 1)
            p, l = softmax(ss[h])
            os_[h] = fold(_dot(p, v32[h]), l)
            if h < HKV - NOM:
                acc = oproj_vpu(os_[h], h, acc)
                accs[h] = acc
        for h in range(HKV - NOM, HKV):
            acc = acc + oproj_mxu(os_[h], h)
        x8 = x8 + _sublane_allsum(acc)
        x8 = x8 + ffn(x8, m)[0]
        return jnp.where(lax.broadcasted_iota(jnp.int32, (8, D), 0) == b, x8, carry)

    xcopy.wait()
    res = lax.fori_loop(0, B, batch, jnp.zeros((8, D), f32))
    o_ref[...] = res[:B].astype(o_ref.dtype)


@jax.jit
def pallas_interleave_layers__gqa_block_cached__dense_activation_silu__decode_kernel(A_x, A_k_cache, A_v_cache, A_wq, A_wo, B_x, B_w1, B_w2):
    k = A_k_cache.reshape(B * HKV, SK, DH)
    v = A_v_cache.reshape(B * HKV, SK, DH)
    any_spec = pl.BlockSpec(memory_space=pl.ANY)
    return pl.pallas_call(
        _kernel,
        out_shape=jax.ShapeDtypeStruct((B, D), A_x.dtype),
        in_specs=[any_spec] * 7,
        out_specs=pl.BlockSpec(memory_space=pltpu.VMEM),
        scratch_shapes=[
            pltpu.VMEM((HKV, SK, DH), bf16),
            pltpu.VMEM((HKV + 1, SK, DH), bf16),
            pltpu.VMEM((HKV, DH // 2, SK), u32),
            pltpu.VMEM((HKV, SK // 2, DH), u32),
            pltpu.VMEM((D, HQ * DH), bf16),
            pltpu.VMEM((HQ * DH, D), bf16),
            pltpu.VMEM((D, F), bf16),
            pltpu.VMEM((F, D), bf16),
            pltpu.VMEM((NQM * REP, D // 2, L), u32),
            pltpu.VMEM((D // L, NOM * HW // 2, L), u32),
            pltpu.VMEM((NFM, D // 2, L), u32),
            pltpu.VMEM((NFM, L // 2, D), u32),
            pltpu.VMEM(((HKV - NQM) * REP, L, D), f32),
            pltpu.VMEM(((HKV - NOM) * HW, D), f32),
            pltpu.VMEM((NFV, L, D), f32),
            pltpu.VMEM((NFV, L, D), f32),
            pltpu.VMEM((HKV, 8, DH), f32),
            pltpu.VMEM((8, SK), f32),
            pltpu.VMEM((HKV, 8, SK), bf16),
            pltpu.VMEM((HKV, 8, DH), f32),
            pltpu.VMEM((8, NFM * L), f32),
            pltpu.VMEM((8, NQM * HW), f32),
            pltpu.VMEM((B, D), bf16),
            pltpu.SMEM((2, SROWS, DH), bf16),
            pltpu.SemaphoreType.DMA((5 + B * NSEM_B,)),
            pltpu.SemaphoreType.DMA((2,)),
        ],
        compiler_params=pltpu.CompilerParams(vmem_limit_bytes=112 * 1024 * 1024, disable_semaphore_checks=True),
    )(A_x.reshape(B, D), k, v, A_wq, A_wo, B_w1, B_w2).reshape(B, 1, D)
```

```python
import dataclasses

import jax
import jax.numpy as jnp
from jax import lax
import jax.experimental.pallas as pl
import jax.experimental.pallas.tpu as pltpu

B, D = 2, 512
HQ, HKV, SK, DH = 32, 8, 8192, 128
REP = HQ // HKV
F = 1792
EPS = 1e-5
SCALE = DH ** -0.5
f32, bf16, u32 = jnp.float32, jnp.bfloat16, jnp.uint32
L = 128
HW = REP * DH
TK = 2048
XR = 768
VCH = (XR, 4096 - XR, 2048, 1024, 1024)
VORD = (1, 2, 3, 0, 4)
XH = 3
VOFF = tuple(sum(VCH[:i]) for i in range(len(VCH)))
NSEM_B = HKV + (HKV - 1) + len(VCH)
NQM = 1
NOM = 2
PIN = 3
SPLIT = 3072
NFV = 6
NFM = F // L - NFV
SB, SH = B - 1, HKV - 2
SROWS = 1024
NSC = SK // SROWS


def _silu(h):
    hh = 0.5 * h
    return hh + hh * jnp.tanh(hh)


def _dot(a, b32):
    return jnp.dot(a, pltpu.bitcast(b32, bf16), preferred_element_type=f32)


def _dot_nt(a, b):
    return lax.dot_general(a, b, (((1,), (1,)), ((), ())), preferred_element_type=f32)


def _sublane_allsum(x):
    x = x + pltpu.roll(x, 4, 0)
    x = x + pltpu.roll(x, 2, 0)
    return x + pltpu.roll(x, 1, 0)


def _kernel(x_hbm, k_hbm, v_hbm, wq_hbm, wo_hbm, w1_hbm, w2_hbm, o_ref,
            k_scr, v_scr, kt_scr, v32, wq_s, wo_s, w1_s, w2_s, wq_r, wo_r, w1_r, w2_r,
            wqt32, wo32, w1t32, w2f32,
            q_scr, s_scr, p_scr, l_scr, cs1_scr, csq_scr, x_ref, sm, sem, ssem):
    def kcopy(b, h):
        return pltpu.make_async_copy(k_hbm.at[b * HKV + h], k_scr.at[h], sem.at[4 + b * NSEM_B + h])

    def vcopy(b, h):
        return pltpu.make_async_copy(v_hbm.at[b * HKV + h], v_scr.at[h], sem.at[4 + b * NSEM_B + HKV + h])

    def vlast(b, c):
        h = HKV - 1
        return pltpu.make_async_copy(v_hbm.at[b * HKV + h, pl.ds(VOFF[c], VCH[c])],
                                     v_scr.at[h, pl.ds(VOFF[c], VCH[c])],
                                     sem.at[4 + b * NSEM_B + 2 * HKV - 1 + c])

    def start_k(b):
        for h in range(HKV):
            kcopy(b, h).start()

    def start_v(b, skip=None):
        for h in range(HKV - 1):
            if h != skip:
                vcopy(b, h).start()
        for c in VORD:
            if not (skip is not None and c == 0):
                vlast(b, c).start()

    def side_in(c, buf):
        return pltpu.make_async_copy(v_hbm.at[SB * HKV + SH, pl.ds(c * SROWS, SROWS)], sm.at[buf], ssem.at[buf])

    def side_out(c, buf):
        return pltpu.make_async_copy(sm.at[buf], v_scr.at[HKV, pl.ds(c * SROWS, SROWS)], ssem.at[buf])

    xtra_in = pltpu.make_async_copy(v_hbm.at[SB * HKV + HKV - 1, pl.ds(0, XR)], sm.at[0, pl.ds(0, XR)], ssem.at[0])
    xtra_out = pltpu.make_async_copy(sm.at[0, pl.ds(0, XR)], v_scr.at[HKV - 1, pl.ds(0, XR)], ssem.at[0])

    def pump(k):
        j = k - 1
        buf = j % 2
        c = 2 * (j // 4) + buf

        @pl.when(jnp.logical_and(j < 2 * NSC, (j // 2) % 2 == 0))
        def _():
            side_in(c, buf).wait()
            side_out(c, buf).start()

        @pl.when(jnp.logical_and(j < 2 * NSC, (j // 2) % 2 == 1))
        def _():
            side_out(c, buf).wait()

            @pl.when(c + 2 < NSC)
            def _():
                side_in(c + 2, buf).start()

            @pl.when(c + 2 == NSC)
            def _():
                xtra_in.start()

    wcopies = [pltpu.make_async_copy(a, b, sem.at[i]) for i, (a, b) in enumerate(
        [(wq_hbm, wq_s), (wo_hbm, wo_s), (w1_hbm, w1_s), (w2_hbm, w2_s)])]
    xcopy = pltpu.make_async_copy(x_hbm, x_ref, sem.at[4 + B * NSEM_B])

    xcopy.start()
    side_in(0, 0).start()
    side_in(1, 1).start()
    for c in wcopies:
        c.start()
    start_k(0)
    start_v(0)

    row = lax.broadcasted_iota(jnp.int32, (8, DH), 0)
    rowr = row % REP
    lo = row < REP
    eye = (lax.broadcasted_iota(jnp.int32, (DH, DH), 0)
           == lax.broadcasted_iota(jnp.int32, (DH, DH), 1)).astype(bf16)
    ones8 = jnp.ones((8, D), bf16)

    def retile(ws, wr, r_lo, r_hi, cols):
        rb = 256
        for j in cols:
            def rbody(i, _, j=j):
                r0 = pl.multiple_of(r_lo + i * rb, rb)
                wr[j, pl.ds(pl.multiple_of(i * (rb // 2), rb // 2), rb // 2), :] = pltpu.bitcast(
                    ws[pl.ds(r0, rb), j * L:(j + 1) * L], u32)
                return 0
            lax.fori_loop(0, (r_hi - r_lo) // rb, rbody, 0)

    wcopies[0].wait()
    retile(wq_s, wq_r, 0, D, range(NQM * REP))
    csq_scr[...] = jnp.dot(ones8, wq_s[:, :NQM * HW], preferred_element_type=f32)
    for j in range(NQM * REP, HQ):
        wqt32[j - NQM * REP] = _dot_nt(eye, wq_s[:, j * L:(j + 1) * L])
    pump(jnp.int32(1))
    wcopies[1].wait()
    retile(wo_s, wo_r, (HKV - NOM) * HW, HKV * HW, range(D // L))

    def obody(i, _):
        r0 = pl.multiple_of(i * L, L)
        wo32[pl.ds(r0, L), :] = wo_s[pl.ds(r0, L), :].astype(f32)
        return 0
    lax.fori_loop(0, (HKV - NOM) * REP, obody, 0)
    wcopies[2].wait()
    retile(w1_s, w1_r, 0, D, range(NFM))
    cs1_scr[...] = jnp.dot(ones8, w1_s[:, :NFM * L], preferred_element_type=f32)
    for j in range(NFV):
        t = _dot_nt(eye, w1_s[:, (NFM + j) * L:(NFM + j + 1) * L])
        w1t32[j] = t - jnp.mean(t, axis=1, keepdims=True)
    pump(jnp.int32(2))
    wcopies[3].wait()

    def w2body(i, _):
        w2_r[i] = pltpu.bitcast(w2_s[pl.ds(pl.multiple_of(i * L, L), L), :], u32)
        return 0
    lax.fori_loop(0, NFM, w2body, 0)
    for j in range(NFV):
        w2f32[j] = w2_s[(NFM + j) * L:(NFM + j + 1) * L, :].astype(f32)

    def qselect(c):
        return jnp.where(rowr == 0, c[0], jnp.where(rowr == 1, c[1], jnp.where(rowr == 2, c[2], c[3])))

    def expand(o):
        return jnp.concatenate([jnp.where(row == r, o, 0.0) for r in range(REP)], axis=1).astype(bf16)

    def oproj_mxu(o, h):
        oh = expand(o)
        hh = (h - (HKV - NOM)) * HW // 2
        return jnp.concatenate([_dot(oh, wo_r[j, hh:hh + HW // 2, :]) for j in range(D // L)], axis=1)

    def dep(x, t):
        return jnp.where(t != t, t, x)

    def lane_fold(w, x):
        prod = w.reshape(L // 8, 8, D) * x[None]
        part = prod[:, :, 0:L]
        for cb in range(1, D // L):
            part = part + prod[:, :, cb * L:(cb + 1) * L]
        return part

    def qhead_vpu(xc, h):
        cs = []
        for r in range(REP):
            t = lane_fold(wqt32[(h - NQM) * REP + r], xc).reshape(L, L).T
            cs.append(_sublane_allsum(jnp.sum(t.reshape(L // 8, 8, L), axis=0)))
        return qselect(cs)

    def oproj_vpu(o, h, acc):
        for r in range(REP):
            ob = jnp.broadcast_to(o[r:r + 1, :], (L, L)).T
            w = wo32[(h * REP + r) * L:(h * REP + r + 1) * L, :]
            prod = jnp.concatenate([ob] * (D // L), axis=1) * w
            t = jnp.sum(prod.reshape(L // 8, 8, D), axis=0)
            acc = t if acc is None else acc + t
        return acc

    def ln_stats(x8, c):
        xb = x8.astype(bf16)
        xs = xb.astype(f32) - c
        ms = jnp.mean(xs, axis=-1, keepdims=True)
        v = jnp.maximum(jnp.mean(xs * xs, axis=-1, keepdims=True) - ms * ms, 0.0)
        return xb, xs - ms, ms + c, lax.rsqrt(v + EPS)

    def ffn(x8, c):
        xb, _, m, rs = ln_stats(x8, c)
        hs = []
        for j in range(NFM):
            hdn = (_dot(xb, w1_r[j]) - m * cs1_scr[:, j * L:(j + 1) * L]) * rs
            hs.append(_silu(hdn).astype(bf16))
        y = _dot(hs[0], w2_r[0])
        for j in range(1, NFM):
            y = y + _dot(hs[j], w2_r[j])
        xr = xb.astype(f32)
        yv = None
        for j in range(NFV):
            hdn = jnp.sum(lane_fold(w1t32[j], xr), axis=-1, keepdims=True) * rs[None]
            t = jnp.sum(w2f32[j].reshape(L // 8, 8, D) * _silu(hdn), axis=0)
            yv = t if yv is None else yv + t
        return y + _sublane_allsum(yv), m

    def softmax(s):
        sp = jnp.concatenate(
            [jnp.where(lo, s[:, 2 * j * L:(2 * j + 1) * L], s[:, (2 * j + 1) * L:(2 * j + 2) * L])
             for j in range(SK // (2 * L))], axis=1)
        m = jnp.broadcast_to(jnp.max(sp, axis=1, keepdims=True), (8, L))
        m = jnp.maximum(m, pltpu.roll(m, REP, 0))
        p = jnp.exp(sp - jnp.concatenate([m] * (SK // (2 * L)), axis=1))
        l = jnp.broadcast_to(jnp.sum(p, axis=1, keepdims=True), (8, L))
        l = l + pltpu.roll(l, REP, 0)
        tiles = []
        for j in range(SK // (2 * L)):
            pj = p[:, j * L:(j + 1) * L]
            tiles += [jnp.where(lo, pj, 0.0), jnp.where(lo, 0.0, pj)]
        return jnp.concatenate(tiles, axis=1).astype(bf16), l

    def fold(o8, l):
        return (o8 + pltpu.roll(o8, REP, 0)) / l

    def batch(b, carry):
        @pl.when(b > 0)
        def _():
            start_v(b, SH)
            pump(2 + 9 * b)

        xf = x_ref[...].astype(f32)
        x8 = jnp.where(b == 0, jnp.broadcast_to(xf[0:1], (8, D)), jnp.broadcast_to(xf[1:2], (8, D)))
        m = jnp.mean(x8, axis=-1, keepdims=True)
        xc = x8 - m
        rs = lax.rsqrt(jnp.mean(xc * xc, axis=-1, keepdims=True) + EPS)
        q8 = jnp.dot(xc.astype(bf16), wq_s[...], preferred_element_type=f32) * (rs * SCALE)
        for h in range(HKV):
            q_scr[h] = qselect([q8[:, (REP * h + r) * DH:(REP * h + r + 1) * DH] for r in range(REP)])

        def kbody(h, _):
            kcopy(b, h).wait()

            @pl.when(h % 2 == 1)
            def _():
                pump(3 + 9 * b + h // 2)
            qh = q_scr[h]
            lhs = jnp.concatenate([jnp.concatenate([qh, qh], axis=0).astype(bf16), eye], axis=0)

            def chunk(c, _):
                off = pl.multiple_of(c * TK, TK)
                r = _dot_nt(lhs, k_scr[h, pl.ds(off, TK), :])
                s_scr[:, pl.ds(off, TK)] = r[:8]
                kt_scr[h, :, pl.ds(off, TK)] = pltpu.bitcast(r[16:].astype(bf16), u32)
                return 0
            lax.fori_loop(0, SK // TK, chunk, 0)
            p, l = softmax(s_scr[...])
            l_scr[h] = l
            p_scr[h] = p
            return 0
        lax.fori_loop(0, HKV, kbody, 0)

        @pl.when(b + 1 < B)
        def _():
            start_k(b + 1)

        def vbody(h, acc):
            side = jnp.logical_and(b == SB, h == SH)

            @pl.when(jnp.logical_not(side))
            def _():
                vcopy(b, h).wait()

            @pl.when(h % 2 == 1)
            def _():
                pump(7 + 9 * b + h // 2)

            @pl.when(jnp.logical_and(b == SB, h == XH))
            def _():
                xtra_in.wait()
                xtra_out.start()
            vv = pltpu.bitcast(v_scr[jnp.where(side, HKV, h)], u32)
            v32[h] = vv
            o = fold(_dot(p_scr[h], vv), l_scr[h])
            wo_h = wo_s[pl.ds(pl.multiple_of(h * HW, HW), HW), :]
            return acc + jnp.dot(expand(o), wo_h, preferred_element_type=f32)
        acc = lax.fori_loop(0, HKV - 1, vbody, jnp.zeros((8, D), f32))
        pump(10 + 9 * b)
        h = HKV - 1
        o = jnp.zeros((8, DH), f32)
        for c in VORD:
            if c == 0:
                @pl.when(b == SB)
                def _():
                    xtra_out.wait()

                @pl.when(b != SB)
                def _():
                    vlast(b, 0).wait()
            else:
                vlast(b, c).wait()
            vv = pltpu.bitcast(v_scr[h, VOFF[c]:VOFF[c] + VCH[c], :], u32)
            v32[h, VOFF[c] // 2:(VOFF[c] + VCH[c]) // 2, :] = vv
            o = o + _dot(p_scr[h, :, VOFF[c]:VOFF[c] + VCH[c]], vv)
        acc = acc + oproj_mxu(fold(o, l_scr[h]), h)
        x8 = x8 + _sublane_allsum(acc)
        y, m = ffn(x8, m)
        x8 = x8 + y

        xb, xc, m, rs = ln_stats(x8, m)
        rq = rs * SCALE
        qs, ss, os_, accs = {}, {}, {}, {}
        for h in range(NQM):
            qraw = qselect([_dot(xb, wq_r[REP * h + r]) for r in range(REP)])
            qcs = qselect([csq_scr[:, (REP * h + r) * L:(REP * h + r + 1) * L] for r in range(REP)])
            qs[h] = (qraw - m * qcs) * rq

        def qk(h):
            pin = accs.get(h - PIN)
            if pin is None:
                return _dot(qs[h].astype(bf16), kt_scr[h])
            q2 = qs[h]
            for j in range(D // L):
                q2 = dep(q2, pin[:, j * L:(j + 1) * L])
            return jnp.concatenate([_dot(qs[h].astype(bf16), kt_scr[h, :, :SPLIT]),
                                    _dot(q2.astype(bf16), kt_scr[h, :, SPLIT:])], axis=1)

        ss[0] = qk(0)
        acc = None
        for h in range(HKV):
            if h + 1 < HKV:
                if h + 1 not in qs:
                    qs[h + 1] = qhead_vpu(xc, h + 1) * rq
                ss[h + 1] = qk(h + 1)
            p, l = softmax(ss[h])
            os_[h] = fold(_dot(p, v32[h]), l)
            if h < HKV - NOM:
                acc = oproj_vpu(os_[h], h, acc)
                accs[h] = acc
        for h in range(HKV - NOM, HKV):
            acc = acc + oproj_mxu(os_[h], h)
        x8 = x8 + _sublane_allsum(acc)
        x8 = x8 + ffn(x8, m)[0]
        return jnp.where(lax.broadcasted_iota(jnp.int32, (8, D), 0) == b, x8, carry)

    xcopy.wait()
    res = lax.fori_loop(0, B, batch, jnp.zeros((8, D), f32))
    o_ref[...] = res[:B].astype(o_ref.dtype)


@jax.jit
def pallas_interleave_layers__gqa_block_cached__dense_activation_silu__decode_kernel(A_x, A_k_cache, A_v_cache, A_wq, A_wo, B_x, B_w1, B_w2):
    k = A_k_cache.reshape(B * HKV, SK, DH)
    v = A_v_cache.reshape(B * HKV, SK, DH)
    any_spec = pl.BlockSpec(memory_space=pl.ANY)
    params = dict(vmem_limit_bytes=112 * 1024 * 1024)
    if any(f.name == "disable_semaphore_checks" for f in dataclasses.fields(pltpu.CompilerParams)):
        params["disable_semaphore_checks"] = True
    return pl.pallas_call(
        _kernel,
        out_shape=jax.ShapeDtypeStruct((B, D), A_x.dtype),
        in_specs=[any_spec] * 7,
        out_specs=pl.BlockSpec(memory_space=pltpu.VMEM),
        scratch_shapes=[
            pltpu.VMEM((HKV, SK, DH), bf16),
            pltpu.VMEM((HKV + 1, SK, DH), bf16),
            pltpu.VMEM((HKV, DH // 2, SK), u32),
            pltpu.VMEM((HKV, SK // 2, DH), u32),
            pltpu.VMEM((D, HQ * DH), bf16),
            pltpu.VMEM((HQ * DH, D), bf16),
            pltpu.VMEM((D, F), bf16),
            pltpu.VMEM((F, D), bf16),
            pltpu.VMEM((NQM * REP, D // 2, L), u32),
            pltpu.VMEM((D // L, NOM * HW // 2, L), u32),
            pltpu.VMEM((NFM, D // 2, L), u32),
            pltpu.VMEM((NFM, L // 2, D), u32),
            pltpu.VMEM(((HKV - NQM) * REP, L, D), f32),
            pltpu.VMEM(((HKV - NOM) * HW, D), f32),
            pltpu.VMEM((NFV, L, D), f32),
            pltpu.VMEM((NFV, L, D), f32),
            pltpu.VMEM((HKV, 8, DH), f32),
            pltpu.VMEM((8, SK), f32),
            pltpu.VMEM((HKV, 8, SK), bf16),
            pltpu.VMEM((HKV, 8, DH), f32),
            pltpu.VMEM((8, NFM * L), f32),
            pltpu.VMEM((8, NQM * HW), f32),
            pltpu.VMEM((B, D), bf16),
            pltpu.SMEM((2, SROWS, DH), bf16),
            pltpu.SemaphoreType.DMA((5 + B * NSEM_B,)),
            pltpu.SemaphoreType.DMA((2,)),
        ],
        compiler_params=pltpu.CompilerParams(**params),
    )(A_x.reshape(B, D), k, v, A_wq, A_wo, B_w1, B_w2).reshape(B, 1, D)
```
